```python
import jax
import jax.numpy as jnp

def _softmax(x, axis=-1):
    return jax.nn.softmax(x, axis=axis)

def _gelu(x):
    return jax.nn.gelu(x, approximate=True)

def _silu(x):
    return jax.nn.silu(x)

def _sigmoid(x):
    return jax.nn.sigmoid(x)

def _layernorm(x, axis=-1, eps=1e-05):
    m = jnp.mean(x, axis=axis, keepdims=True)
    v = jnp.var(x, axis=axis, keepdims=True)
    return (x - m) / jnp.sqrt(v + eps)

def _scatter_add(tgt, idx, src, axis=0):
    return tgt.at[idx].add(src)

def _segment_sum(src, seg, n):
    return jax.ops.segment_sum(src, seg, n)

class _Rng:

    def __init__(self, key):
        self._k = key

    def _next(self):
        self._k, sub = jax.random.split(self._k)
        return sub

    def normal(self, shape):
        return jax.random.normal(self._next(), shape, dtype=jnp.bfloat16)

    def randint(self, lo, hi, shape):
        return jax.random.randint(self._next(), shape, lo, hi, dtype=jnp.int32)

    def uniform(self, shape, lo=0.0, hi=1.0):
        return jax.random.uniform(self._next(), shape, jnp.bfloat16, lo, hi)

    def permutation(self, n):
        return jax.random.permutation(self._next(), n)
kernel_name = 'adaLN_cond__compressed_kv_cla__glu_gated_geglu__decode'

def setup_inputs():
    _rng = _Rng(jax.random.key(int.from_bytes(__import__("os").urandom(4), "little")))
    _w = lambda a: (lambda t: t.astype(jnp.bfloat16) if jnp.issubdtype(t.dtype, jnp.floating) else t)(jnp.asarray(a))

    def _A_setup():
        B, H, Sq, Sk, D, M = (1, 32, 1, 32768, 128, 512)
        Dc = 4 * D
        return {'x': _w((lambda *s: _rng.normal(s) * 0.05)(B, Sq, M)), 'c_kv': _w((lambda *s: _rng.normal(s) * 0.05)(B, Sk, Dc)), 'w_q': _w((lambda *s: _rng.normal(s) * 0.05)(M, H, D) * M ** (-0.5)), 'w_uk': _w((lambda *s: _rng.normal(s) * 0.05)(Dc, H, D) * Dc ** (-0.5)), 'w_uv': _w((lambda *s: _rng.normal(s) * 0.05)(Dc, H, D) * Dc ** (-0.5)), 'w_o': _w((lambda *s: _rng.normal(s) * 0.05)(H, D, M) * (H * D) ** (-0.5))}
    _A_in = _A_setup()

    def _B_setup():
        B, S, Dm, Df = (1, 1, 512, 1792)
        return {'x': _w((lambda *s: _rng.normal(s) * 0.05)(B, S, Dm)), 'w_gate': _w((lambda *s: _rng.normal(s) * 0.05)(Dm, Df) * Dm ** (-0.5)), 'w_up': _w((lambda *s: _rng.normal(s) * 0.05)(Dm, Df) * Dm ** (-0.5)), 'w_down': _w((lambda *s: _rng.normal(s) * 0.05)(Df, Dm) * Df ** (-0.5))}
    _B_in = _B_setup()
    return {'A_x': _A_in['x'], 'A_c_kv': _A_in['c_kv'], 'A_w_q': _A_in['w_q'], 'A_w_uk': _A_in['w_uk'], 'A_w_uv': _A_in['w_uv'], 'A_w_o': _A_in['w_o'], 'B_x': _B_in['x'], 'B_w_gate': _B_in['w_gate'], 'B_w_up': _B_in['w_up'], 'B_w_down': _B_in['w_down'], 'c': _w((lambda *s: _rng.normal(s) * 0.05)(1, 512)), 'w_mod': _w((lambda *s: _rng.normal(s) * 0.05)(512, 6 * 512) * 512 ** (-0.5))}

def reference(A_x, A_c_kv, A_w_q, A_w_uk, A_w_uv, A_w_o, B_x, B_w_gate, B_w_up, B_w_down, c, w_mod):

    def _A_ref(x, c_kv, w_q, w_uk, w_uv, w_o):
        B, Sq, M = (x.shape[0], x.shape[1], x.shape[2])
        Sk = c_kv.shape[1]
        H, D = (w_q.shape[1], w_q.shape[2])
        q = jnp.einsum('bqm,mhd->bhqd', x, w_q)
        k = jnp.einsum('bkc,chd->bhkd', c_kv, w_uk)
        v = jnp.einsum('bkc,chd->bhkd', c_kv, w_uv)
        scores = jnp.einsum('bhqd,bhkd->bhqk', q, k) * D ** (-0.5)
        off = Sk - Sq
        qi = jnp.arange(Sq)[:, None]
        kj = jnp.arange(Sk)[None, :]
        cmask = kj <= qi + off
        scores = jnp.where(cmask[None, None], scores, -1000000000.0)
        p = _softmax(scores, axis=-1)
        ctx = jnp.einsum('bhqk,bhkd->bhqd', p, v)
        return jnp.einsum('bhqd,hdm->bqm', ctx, w_o)

    def _B_ref(x, w_gate, w_up, w_down):
        g = jnp.einsum('bsd,df->bsf', x, w_gate)
        u = jnp.einsum('bsd,df->bsf', x, w_up)
        h = _gelu(g) * u
        return jnp.einsum('bsf,fd->bsd', h, w_down)
    x = A_x
    mod = (_silu(c) @ w_mod).reshape(c.shape[0], 6, 1, -1)
    sa, ca, ga, sb, cb, gb = (mod[:, 0].copy(), mod[:, 1].copy(), mod[:, 2].copy(), mod[:, 3].copy(), mod[:, 4].copy(), mod[:, 5].copy())
    h = _layernorm(x, axis=-1) * (1 + ca) + sa
    x = x + ga * _A_ref(h, A_c_kv, A_w_q, A_w_uk, A_w_uv, A_w_o)
    h = _layernorm(x, axis=-1) * (1 + cb) + sb
    x = x + gb * _B_ref(h, B_w_gate, B_w_up, B_w_down)
    return x
```

```python
import functools

import jax
import jax.numpy as jnp
from jax import lax
import jax.experimental.pallas as pl
import jax.experimental.pallas.tpu as pltpu

_NN = (((1,), (0,)), ((), ()))
_NT = (((1,), (1,)), ((), ()))
_F32 = jnp.float32
_BF16 = jnp.bfloat16

_KV_DMA_ROWS = 8192
_TK = 2048
_WD_SPLITS = (0, 1280, 1536, 1664, 1792)


def _dot(a, b, dims=_NN):
    return lax.dot_general(a, b, dims, preferred_element_type=_F32)


def _layernorm(x, eps=1e-5):
    m = jnp.mean(x, axis=-1, keepdims=True)
    xc = x - m
    v = jnp.mean(xc * xc, axis=-1, keepdims=True)
    return xc / jnp.sqrt(v + eps)


def _kernel(x_hbm, c_hbm, wmod_hbm, wq_hbm, wuk_hbm, ckv_hbm, wuv_hbm, wo_hbm,
            wg_hbm, wu_hbm, wd_hbm,
            o_ref,
            x_v, c_v, wmod_v, wq_v, wuk_v, ckv_v, wuv_v, wo_v, wg_v, wu_v, wd_v,
            e_v, qa_v, acc_v, m_v, l_v, sems, kv_sems, wd_sems,
            *, H, D, M, DC, SK):
    n_kv = SK // _KV_DMA_ROWS
    n_wd = len(_WD_SPLITS) - 1
    G = 128 * H

    def whole(src, dst, k):
        return pltpu.make_async_copy(src, dst, sems.at[k])

    def kv_copy(j):
        r = j * _KV_DMA_ROWS
        if not isinstance(j, int):
            r = pl.multiple_of(r, _KV_DMA_ROWS)
        return pltpu.make_async_copy(ckv_hbm.at[pl.ds(r, _KV_DMA_ROWS)],
                                     ckv_v.at[pl.ds(r, _KV_DMA_ROWS)], kv_sems.at[j])

    def wd_copy(j):
        r0, r1 = _WD_SPLITS[j], _WD_SPLITS[j + 1]
        return pltpu.make_async_copy(wd_hbm.at[pl.ds(r0, r1 - r0)],
                                     wd_v.at[pl.ds(r0, r1 - r0)], wd_sems.at[j])

    cp_wmod = whole(wmod_hbm, wmod_v, 0)
    cp_x = whole(x_hbm, x_v, 1)
    cp_c = whole(c_hbm, c_v, 2)
    cp_wq = whole(wq_hbm, wq_v, 3)
    cp_wuk = whole(wuk_hbm, wuk_v, 4)
    cp_wuv = whole(wuv_hbm, wuv_v, 5)
    cp_wo = whole(wo_hbm, wo_v, 6)
    cp_wg = whole(wg_hbm, wg_v, 7)
    cp_wu = whole(wu_hbm, wu_v, 8)

    for cp in (cp_wmod, cp_x, cp_c, cp_wq, cp_wuk):
        cp.start()
    for j in range(n_kv):
        kv_copy(j).start()
    for cp in (cp_wuv, cp_wo, cp_wg, cp_wu):
        cp.start()
    for j in range(n_wd):
        wd_copy(j).start()

    CH = 1024
    for b in range(G // CH):
        row = lax.broadcasted_iota(jnp.int32, (128, CH), 0)
        col = lax.broadcasted_iota(jnp.int32, (128, CH), 1) + b * CH
        e_v[:, b * CH:(b + 1) * CH] = jnp.where(col // H == row, 1.0, 0.0).astype(_BF16)
    hsel = (lax.broadcasted_iota(jnp.int32, (H, CH), 1) % H
            == lax.broadcasted_iota(jnp.int32, (H, CH), 0))

    def expand_contract(lhs, w_ref):
        out = jnp.zeros((H, D), _F32)
        for a in range(lhs.shape[1] // 128):
            la = lhs[:, a * 128:(a + 1) * 128]
            for b in range(G // CH):
                t = _dot(la, e_v[:, b * CH:(b + 1) * CH])
                t = jnp.where(hsel, t, 0.0).astype(_BF16)
                r0 = a * G + b * CH
                out = out + _dot(t, w_ref[r0:r0 + CH, :])
        return out

    acc_v[...] = jnp.zeros_like(acc_v)
    m_v[...] = jnp.full_like(m_v, -jnp.inf)
    l_v[...] = jnp.zeros_like(l_v)

    cp_wmod.wait()
    cp_x.wait()
    cp_c.wait()
    c = c_v[...].astype(_F32)
    sc = (c * jax.nn.sigmoid(c)).astype(_BF16)
    mod = _dot(sc, wmod_v[...])
    sa, ca, ga, sb, cb, gb = [mod[:, i * M:(i + 1) * M] for i in range(6)]
    x = x_v[...].astype(_F32)
    h1 = (_layernorm(x) * (1.0 + ca) + sa).astype(_BF16)

    cp_wq.wait()
    q = expand_contract(jnp.broadcast_to(h1, (H, M)), wq_v)
    q = q.astype(_BF16)

    cp_wuk.wait()
    scale = D ** (-0.5)
    for a in range(DC // 128):
        qa = jnp.zeros((H, 128), _F32)
        for b in range(G // CH):
            r0 = a * G + b * CH
            t = _dot(q, wuk_v[r0:r0 + CH, :], _NT)
            t = jnp.where(hsel, t * scale, 0.0).astype(_BF16)
            qa = qa + _dot(t, e_v[:, b * CH:(b + 1) * CH], _NT)
        qa_v[:, a * 128:(a + 1) * 128] = qa.astype(_BF16)

    steps_per_dma = _KV_DMA_ROWS // _TK

    def attn_step(i, carry):
        @pl.when(i % steps_per_dma == 0)
        def _():
            kv_copy(i // steps_per_dma).wait()

        off = pl.multiple_of(i * _TK, _TK)
        ck = ckv_v[pl.ds(off, _TK), :]
        s = _dot(qa_v[...], ck, _NT)
        m_prev = m_v[...]
        m_new = jnp.maximum(m_prev, jnp.max(s, axis=1, keepdims=True))
        alpha = jnp.exp(m_prev - m_new)
        p = jnp.exp(s - m_new[:, 0:1])
        ps = p[:, 0:128]
        for j in range(1, _TK // 128):
            ps = ps + p[:, j * 128:(j + 1) * 128]
        l_v[...] = l_v[...] * alpha + ps
        m_v[...] = m_new
        acc_v[...] = acc_v[...] * alpha[:, 0:1] + _dot(p.astype(_BF16), ck)
        return carry

    lax.fori_loop(0, SK // _TK, attn_step, 0)

    l = jnp.sum(l_v[...], axis=1, keepdims=True)
    ctx_c = (acc_v[...] / l).astype(_BF16)

    cp_wuv.wait()
    ctx = expand_contract(ctx_c, wuv_v)

    rid = lax.broadcasted_iota(jnp.int32, (16, D), 0)
    blocks = []
    for h in range(H):
        g0 = (h // 16) * 16
        blocks.append(jnp.where(rid == h % 16, ctx[g0:g0 + 16, :], 0.0).astype(_BF16))
    ctx_bd = jnp.concatenate(blocks, axis=1)
    cp_wo.wait()
    attn = jnp.sum(_dot(ctx_bd, wo_v[...]), axis=0, keepdims=True)
    x1 = x + ga * attn

    h2 = (_layernorm(x1) * (1.0 + cb) + sb).astype(_BF16)
    cp_wg.wait()
    g = jax.nn.gelu(_dot(h2, wg_v[...]), approximate=True)
    cp_wu.wait()
    hh = (g * _dot(h2, wu_v[...])).astype(_BF16)
    y = jnp.zeros((1, M), _F32)
    for j in range(n_wd):
        r0, r1 = _WD_SPLITS[j], _WD_SPLITS[j + 1]
        wd_copy(j).wait()
        y = y + _dot(hh[:, r0:r1], wd_v[r0:r1, :])
    o_ref[...] = (x1 + gb * y).astype(o_ref.dtype)


@jax.jit
def pallas_adaLN_cond__compressed_kv_cla__glu_gated_geglu__decode_kernel(
    A_x: jax.Array,
    A_c_kv: jax.Array,
    A_w_q: jax.Array,
    A_w_uk: jax.Array,
    A_w_uv: jax.Array,
    A_w_o: jax.Array,
    B_x: jax.Array,
    B_w_gate: jax.Array,
    B_w_up: jax.Array,
    B_w_down: jax.Array,
    c: jax.Array,
    w_mod: jax.Array,
):
    del B_x
    B, SQ, M = A_x.shape
    SK, DC = A_c_kv.shape[1], A_c_kv.shape[2]
    H, D = A_w_q.shape[1], A_w_q.shape[2]
    assert B == 1 and SQ == 1 and c.shape[0] == 1
    assert B_w_down.shape[0] == _WD_SPLITS[-1]

    operands = (
        A_x.reshape(1, M),
        c,
        w_mod,
        A_w_q.reshape(M * H, D),
        A_w_uk.reshape(DC * H, D),
        A_c_kv.reshape(SK, DC),
        A_w_uv.reshape(DC * H, D),
        A_w_o.reshape(H * D, M),
        B_w_gate,
        B_w_up,
        B_w_down,
    )
    scratch = [pltpu.VMEM(a.shape, a.dtype) for a in operands] + [
        pltpu.VMEM((128, 128 * H), _BF16),
        pltpu.VMEM((H, DC), _BF16),
        pltpu.VMEM((H, DC), _F32),
        pltpu.VMEM((H, 128), _F32),
        pltpu.VMEM((H, 128), _F32),
        pltpu.SemaphoreType.DMA((9,)),
        pltpu.SemaphoreType.DMA((SK // _KV_DMA_ROWS,)),
        pltpu.SemaphoreType.DMA((len(_WD_SPLITS) - 1,)),
    ]
    out = pl.pallas_call(
        functools.partial(_kernel, H=H, D=D, M=M, DC=DC, SK=SK),
        out_shape=jax.ShapeDtypeStruct((1, M), A_x.dtype),
        in_specs=[pl.BlockSpec(memory_space=pl.ANY)] * len(operands),
        out_specs=pl.BlockSpec(memory_space=pltpu.VMEM),
        scratch_shapes=scratch,
        compiler_params=pltpu.CompilerParams(vmem_limit_bytes=100 * 1024 * 1024),
    )(*operands)
    return out.reshape(B, SQ, M)
```

```python
import functools

import jax
import jax.numpy as jnp
from jax import lax
import jax.experimental.pallas as pl
import jax.experimental.pallas.tpu as pltpu

_NN = (((1,), (0,)), ((), ()))
_NT = (((1,), (1,)), ((), ()))
_F32 = jnp.float32
_BF16 = jnp.bfloat16

_KV_DMA_ROWS = 8192
_TK = 2048
_WD_SPLITS = (0, 1280, 1536, 1664, 1792)


def _dot(a, b, dims=_NN):
    return lax.dot_general(a, b, dims, preferred_element_type=_F32)


def _layernorm(x, eps=1e-5):
    m = jnp.mean(x, axis=-1, keepdims=True)
    xc = x - m
    v = jnp.mean(xc * xc, axis=-1, keepdims=True)
    return xc / jnp.sqrt(v + eps)


def _kernel(x_hbm, c_hbm, wmod_hbm, wq_hbm, wuk_hbm, ckv_hbm, wuv_hbm, wo_hbm,
            wg_hbm, wu_hbm, wd_hbm,
            o_ref,
            x_v, c_v, wmod_v, wq_v, wuk_v, ckv_v, wuv_v, wo_v, wg_v, wu_v, wd_v,
            e_v, qa_v, acc_v, m_v, l_v, sems,
            *, H, D, M, DC, SK):
    n_kv = SK // _KV_DMA_ROWS
    n_wd = len(_WD_SPLITS) - 1
    G = 128 * H

    def whole(src, dst, k):
        return pltpu.make_async_copy(src, dst, sems.at[k])

    def kv_copy(j):
        r = j * _KV_DMA_ROWS
        if not isinstance(j, int):
            r = pl.multiple_of(r, _KV_DMA_ROWS)
        return pltpu.make_async_copy(ckv_hbm.at[pl.ds(r, _KV_DMA_ROWS)],
                                     ckv_v.at[pl.ds(r, _KV_DMA_ROWS)], sems.at[9 + j])

    def wd_copy(j):
        r0, r1 = _WD_SPLITS[j], _WD_SPLITS[j + 1]
        return pltpu.make_async_copy(wd_hbm.at[pl.ds(r0, r1 - r0)],
                                     wd_v.at[pl.ds(r0, r1 - r0)], sems.at[9 + n_kv + j])

    cp_wmod = whole(wmod_hbm, wmod_v, 0)
    cp_x = whole(x_hbm, x_v, 1)
    cp_c = whole(c_hbm, c_v, 2)
    cp_wq = whole(wq_hbm, wq_v, 3)
    cp_wuk = whole(wuk_hbm, wuk_v, 4)
    cp_wuv = whole(wuv_hbm, wuv_v, 5)
    cp_wo = whole(wo_hbm, wo_v, 6)
    cp_wg = whole(wg_hbm, wg_v, 7)
    cp_wu = whole(wu_hbm, wu_v, 8)

    for cp in (cp_wmod, cp_x, cp_c, cp_wq, cp_wuk):
        cp.start()
    for j in range(n_kv):
        kv_copy(j).start()
    for cp in (cp_wuv, cp_wo, cp_wg, cp_wu):
        cp.start()
    for j in range(n_wd):
        wd_copy(j).start()

    CH = 1024
    for b in range(G // CH):
        row = lax.broadcasted_iota(jnp.int32, (128, CH), 0)
        col = lax.broadcasted_iota(jnp.int32, (128, CH), 1) + b * CH
        e_v[:, b * CH:(b + 1) * CH] = jnp.where(col // H == row, 1.0, 0.0).astype(_BF16)
    hsel = (lax.broadcasted_iota(jnp.int32, (H, CH), 1) % H
            == lax.broadcasted_iota(jnp.int32, (H, CH), 0))

    def expand_contract(lhs, w_ref):
        out = jnp.zeros((H, D), _F32)
        for a in range(lhs.shape[1] // 128):
            la = lhs[:, a * 128:(a + 1) * 128]
            for b in range(G // CH):
                t = _dot(la, e_v[:, b * CH:(b + 1) * CH])
                t = jnp.where(hsel, t, 0.0).astype(_BF16)
                r0 = a * G + b * CH
                out = out + _dot(t, w_ref[r0:r0 + CH, :])
        return out

    acc_v[...] = jnp.zeros_like(acc_v)
    m_v[...] = jnp.full_like(m_v, -jnp.inf)
    l_v[...] = jnp.zeros_like(l_v)

    cp_wmod.wait()
    cp_x.wait()
    cp_c.wait()
    c = c_v[...].astype(_F32)
    sc = (c * jax.nn.sigmoid(c)).astype(_BF16)
    mod = _dot(sc, wmod_v[...])
    sa, ca, ga, sb, cb, gb = [mod[:, i * M:(i + 1) * M] for i in range(6)]
    x = x_v[...].astype(_F32)
    h1 = (_layernorm(x) * (1.0 + ca) + sa).astype(_BF16)

    cp_wq.wait()
    q = expand_contract(jnp.broadcast_to(h1, (H, M)), wq_v)
    q = q.astype(_BF16)

    cp_wuk.wait()
    scale = D ** (-0.5)
    for a in range(DC // 128):
        qa = jnp.zeros((H, 128), _F32)
        for b in range(G // CH):
            r0 = a * G + b * CH
            t = _dot(q, wuk_v[r0:r0 + CH, :], _NT)
            t = jnp.where(hsel, t * scale, 0.0).astype(_BF16)
            qa = qa + _dot(t, e_v[:, b * CH:(b + 1) * CH], _NT)
        qa_v[:, a * 128:(a + 1) * 128] = qa.astype(_BF16)

    steps_per_dma = _KV_DMA_ROWS // _TK

    def attn_step(i, carry):
        @pl.when(i % steps_per_dma == 0)
        def _():
            kv_copy(i // steps_per_dma).wait()

        off = pl.multiple_of(i * _TK, _TK)
        ck = ckv_v[pl.ds(off, _TK), :]
        s = _dot(qa_v[...], ck, _NT)
        m_prev = m_v[...]
        m_new = jnp.maximum(m_prev, jnp.max(s, axis=1, keepdims=True))
        alpha = jnp.exp(m_prev - m_new)
        p = jnp.exp(s - m_new[:, 0:1])
        ps = p[:, 0:128]
        for j in range(1, _TK // 128):
            ps = ps + p[:, j * 128:(j + 1) * 128]
        l_v[...] = l_v[...] * alpha + ps
        m_v[...] = m_new
        acc_v[...] = acc_v[...] * alpha[:, 0:1] + _dot(p.astype(_BF16), ck)
        return carry

    lax.fori_loop(0, SK // _TK, attn_step, 0)

    l = jnp.sum(l_v[...], axis=1, keepdims=True)
    ctx_c = (acc_v[...] / l).astype(_BF16)

    cp_wuv.wait()
    ctx = expand_contract(ctx_c, wuv_v)

    rid = lax.broadcasted_iota(jnp.int32, (16, D), 0)
    blocks = []
    for h in range(H):
        g0 = (h // 16) * 16
        blocks.append(jnp.where(rid == h % 16, ctx[g0:g0 + 16, :], 0.0).astype(_BF16))
    ctx_bd = jnp.concatenate(blocks, axis=1)
    cp_wo.wait()
    attn = jnp.sum(_dot(ctx_bd, wo_v[...]), axis=0, keepdims=True)
    x1 = x + ga * attn

    h2 = (_layernorm(x1) * (1.0 + cb) + sb).astype(_BF16)
    cp_wg.wait()
    g = jax.nn.gelu(_dot(h2, wg_v[...]), approximate=True)
    cp_wu.wait()
    hh = (g * _dot(h2, wu_v[...])).astype(_BF16)
    y = jnp.zeros((1, M), _F32)
    for j in range(n_wd):
        r0, r1 = _WD_SPLITS[j], _WD_SPLITS[j + 1]
        wd_copy(j).wait()
        y = y + _dot(hh[:, r0:r1], wd_v[r0:r1, :])
    o_ref[...] = (x1 + gb * y).astype(o_ref.dtype)


@jax.jit
def pallas_adaLN_cond__compressed_kv_cla__glu_gated_geglu__decode_kernel(
    A_x: jax.Array,
    A_c_kv: jax.Array,
    A_w_q: jax.Array,
    A_w_uk: jax.Array,
    A_w_uv: jax.Array,
    A_w_o: jax.Array,
    B_x: jax.Array,
    B_w_gate: jax.Array,
    B_w_up: jax.Array,
    B_w_down: jax.Array,
    c: jax.Array,
    w_mod: jax.Array,
):
    del B_x
    B, SQ, M = A_x.shape
    SK, DC = A_c_kv.shape[1], A_c_kv.shape[2]
    H, D = A_w_q.shape[1], A_w_q.shape[2]
    assert B == 1 and SQ == 1 and c.shape[0] == 1
    assert B_w_down.shape[0] == _WD_SPLITS[-1]

    operands = (
        A_x.reshape(1, M),
        c,
        w_mod,
        A_w_q.reshape(M * H, D),
        A_w_uk.reshape(DC * H, D),
        A_c_kv.reshape(SK, DC),
        A_w_uv.reshape(DC * H, D),
        A_w_o.reshape(H * D, M),
        B_w_gate,
        B_w_up,
        B_w_down,
    )
    scratch = [pltpu.VMEM(a.shape, a.dtype) for a in operands] + [
        pltpu.VMEM((128, 128 * H), _BF16),
        pltpu.VMEM((H, DC), _BF16),
        pltpu.VMEM((H, DC), _F32),
        pltpu.VMEM((H, 128), _F32),
        pltpu.VMEM((H, 128), _F32),
        pltpu.SemaphoreType.DMA((9 + SK // _KV_DMA_ROWS + len(_WD_SPLITS) - 1,)),
    ]
    out = pl.pallas_call(
        functools.partial(_kernel, H=H, D=D, M=M, DC=DC, SK=SK),
        out_shape=jax.ShapeDtypeStruct((1, M), A_x.dtype),
        in_specs=[pl.BlockSpec(memory_space=pl.ANY)] * len(operands),
        out_specs=pl.BlockSpec(memory_space=pltpu.VMEM),
        scratch_shapes=scratch,
        compiler_params=pltpu.CompilerParams(vmem_limit_bytes=100 * 1024 * 1024),
    )(*operands)
    return out.reshape(B, SQ, M)
```

```python
import functools

import jax
import jax.numpy as jnp
from jax import lax
import jax.experimental.pallas as pl
import jax.experimental.pallas.tpu as pltpu

_NN = (((1,), (0,)), ((), ()))
_NT = (((1,), (1,)), ((), ()))
_F32 = jnp.float32
_BF16 = jnp.bfloat16

_KV_DMA_ROWS = 8192
_TK = 2048
_WD_SPLITS = (0, 1024, 1408, 1536, 1664, 1760, 1792)
_VPU_ROW0 = 1408
_N_WHOLE = 9


def _dot(a, b, dims=_NN):
    return lax.dot_general(a, b, dims, preferred_element_type=_F32)


def _layernorm(x, eps=1e-5):
    m = jnp.mean(x, axis=-1, keepdims=True)
    xc = x - m
    v = jnp.mean(xc * xc, axis=-1, keepdims=True)
    return xc / jnp.sqrt(v + eps)


def _tree_sum(parts):
    while len(parts) > 1:
        parts = [parts[i] + parts[i + 1] if i + 1 < len(parts) else parts[i]
                 for i in range(0, len(parts), 2)]
    return parts[0]


def _kernel(*refs, SK, **dims):
    n_sems = _N_WHOLE + SK // _KV_DMA_ROWS + len(_WD_SPLITS) - 1
    pl.run_scoped(lambda sems: _body(*refs, sems, SK=SK, **dims),
                  pltpu.SemaphoreType.DMA((n_sems,)))


def _body(x_hbm, c_hbm, wmod_hbm, wq_hbm, wuk_hbm, ckv_hbm, wuv_hbm, wo_hbm,
          wg_hbm, wu_hbm, wd_hbm,
          o_ref,
          x_v, c_v, wmod_v, wq_v, wuk_v, ckv_v, wuv_v, wo_v, wg_v, wu_v, wd_v,
          e_v, qa_v, acc_v, m_v, l_v, hcol_v, hg_v, sems,
          *, H, D, M, DC, SK):
    n_kv = SK // _KV_DMA_ROWS
    n_wd = len(_WD_SPLITS) - 1
    G = 128 * H

    def whole(src, dst, k):
        return pltpu.make_async_copy(src, dst, sems.at[k])

    def kv_copy(j):
        r = j * _KV_DMA_ROWS
        if not isinstance(j, int):
            r = pl.multiple_of(r, _KV_DMA_ROWS)
        return pltpu.make_async_copy(ckv_hbm.at[pl.ds(r, _KV_DMA_ROWS)],
                                     ckv_v.at[pl.ds(r, _KV_DMA_ROWS)],
                                     sems.at[_N_WHOLE + j])

    def wd_copy(j):
        r0, r1 = _WD_SPLITS[j], _WD_SPLITS[j + 1]
        return pltpu.make_async_copy(wd_hbm.at[pl.ds(r0, r1 - r0)],
                                     wd_v.at[pl.ds(r0, r1 - r0)],
                                     sems.at[_N_WHOLE + n_kv + j])

    cp_wmod = whole(wmod_hbm, wmod_v, 0)
    cp_x = whole(x_hbm, x_v, 1)
    cp_c = whole(c_hbm, c_v, 2)
    cp_wq = whole(wq_hbm, wq_v, 3)
    cp_wuk = whole(wuk_hbm, wuk_v, 4)
    cp_wuv = whole(wuv_hbm, wuv_v, 5)
    cp_wo = whole(wo_hbm, wo_v, 6)
    cp_wg = whole(wg_hbm, wg_v, 7)
    cp_wu = whole(wu_hbm, wu_v, 8)

    for cp in (cp_wmod, cp_x, cp_c, cp_wq, cp_wuk):
        cp.start()
    for j in range(n_kv):
        kv_copy(j).start()
    for cp in (cp_wuv, cp_wo, cp_wg, cp_wu):
        cp.start()
    for j in range(n_wd):
        wd_copy(j).start()

    CH = 1024
    for b in range(G // CH):
        row = lax.broadcasted_iota(jnp.int32, (128, CH), 0)
        col = lax.broadcasted_iota(jnp.int32, (128, CH), 1) + b * CH
        e_v[:, b * CH:(b + 1) * CH] = jnp.where(col // H == row, 1.0, 0.0).astype(_BF16)
    hsel = (lax.broadcasted_iota(jnp.int32, (H, CH), 1) % H
            == lax.broadcasted_iota(jnp.int32, (H, CH), 0))

    def expand_contract(lhs, w_ref):
        out = jnp.zeros((H, D), _F32)
        for a in range(lhs.shape[1] // 128):
            la = lhs[:, a * 128:(a + 1) * 128]
            for b in range(G // CH):
                t = _dot(la, e_v[:, b * CH:(b + 1) * CH])
                t = jnp.where(hsel, t, 0.0).astype(_BF16)
                r0 = a * G + b * CH
                out = out + _dot(t, w_ref[r0:r0 + CH, :])
        return out

    acc_v[...] = jnp.zeros_like(acc_v)
    m_v[...] = jnp.full_like(m_v, -jnp.inf)
    l_v[...] = jnp.zeros_like(l_v)

    cp_wmod.wait()
    cp_x.wait()
    cp_c.wait()
    c = c_v[...].astype(_F32)
    sc = (c * jax.nn.sigmoid(c)).astype(_BF16)
    mod = _dot(sc, wmod_v[...])
    sa, ca, ga, sb, cb, gb = [mod[:, i * M:(i + 1) * M] for i in range(6)]
    x = x_v[...].astype(_F32)
    h1 = (_layernorm(x) * (1.0 + ca) + sa).astype(_BF16)

    cp_wq.wait()
    q = expand_contract(jnp.broadcast_to(h1, (H, M)), wq_v)
    q = q.astype(_BF16)

    cp_wuk.wait()
    scale = D ** (-0.5)
    for a in range(DC // 128):
        qa = jnp.zeros((H, 128), _F32)
        for b in range(G // CH):
            r0 = a * G + b * CH
            t = _dot(q, wuk_v[r0:r0 + CH, :], _NT)
            t = jnp.where(hsel, t * scale, 0.0).astype(_BF16)
            qa = qa + _dot(t, e_v[:, b * CH:(b + 1) * CH], _NT)
        qa_v[:, a * 128:(a + 1) * 128] = qa.astype(_BF16)

    steps_per_dma = _KV_DMA_ROWS // _TK

    def attn_step(i, carry):
        @pl.when(i % steps_per_dma == 0)
        def _():
            kv_copy(i // steps_per_dma).wait()

        off = pl.multiple_of(i * _TK, _TK)
        ck = ckv_v[pl.ds(off, _TK), :]
        s = _dot(qa_v[...], ck, _NT)
        m_prev = m_v[...]
        m_new = jnp.maximum(m_prev, jnp.max(s, axis=1, keepdims=True))
        alpha = jnp.exp(m_prev - m_new)
        p = jnp.exp(s - m_new[:, 0:1])
        ps = p[:, 0:128]
        for j in range(1, _TK // 128):
            ps = ps + p[:, j * 128:(j + 1) * 128]
        l_v[...] = l_v[...] * alpha + ps
        m_v[...] = m_new
        acc_v[...] = acc_v[...] * alpha[:, 0:1] + _dot(p.astype(_BF16), ck)
        return carry

    lax.fori_loop(0, SK // _TK, attn_step, 0)

    l = jnp.sum(l_v[...], axis=1, keepdims=True)
    ctx_c = (acc_v[...] / l).astype(_BF16)

    cp_wuv.wait()
    ctx = expand_contract(ctx_c, wuv_v)

    rid = lax.broadcasted_iota(jnp.int32, (16, D), 0)
    blocks = []
    for h in range(H):
        g0 = (h // 16) * 16
        blocks.append(jnp.where(rid == h % 16, ctx[g0:g0 + 16, :], 0.0).astype(_BF16))
    ctx_bd = jnp.concatenate(blocks, axis=1)
    cp_wo.wait()
    attn = jnp.sum(_dot(ctx_bd, wo_v[...]), axis=0, keepdims=True)
    x1 = x + ga * attn

    h2 = (_layernorm(x1) * (1.0 + cb) + sb).astype(_BF16)
    cp_wg.wait()
    g = jax.nn.gelu(_dot(h2, wg_v[...]), approximate=True)
    cp_wu.wait()
    hh = (g * _dot(h2, wu_v[...])).astype(_BF16)

    for r in range(_VPU_ROW0, _WD_SPLITS[-1], 128):
        hcol_v[r - _VPU_ROW0:r - _VPU_ROW0 + 128, :] = jnp.transpose(
            jnp.broadcast_to(hh[:, r:r + 128].astype(_F32), (128, 128)))

    def hcol(r):
        hc = hcol_v[r - _VPU_ROW0:r - _VPU_ROW0 + 8, :]
        return jnp.concatenate([hc] * (M // 128), axis=1)

    gb8 = jnp.broadcast_to(gb, (8, M))
    r_last = _WD_SPLITS[-2]
    for r in range(r_last, _WD_SPLITS[-1], 8):
        hg_v[r - r_last:r - r_last + 8, :] = hcol(r) * gb8
    row0 = lax.broadcasted_iota(jnp.int32, (8, M), 0) == 0

    y = None
    y8 = None
    for j in range(n_wd - 1):
        r0, r1 = _WD_SPLITS[j], _WD_SPLITS[j + 1]
        wd_copy(j).wait()
        if r0 < _VPU_ROW0:
            t = _dot(hh[:, r0:r1], wd_v[r0:r1, :])
            y = t if y is None else t + y
            if r1 >= _VPU_ROW0:
                pre8 = jnp.where(row0, jnp.broadcast_to(x1 + gb * y, (8, M)), 0.0)
        else:
            y8 = _tree_sum(([] if y8 is None else [y8]) + [
                wd_v[r:r + 8, :].astype(_F32) * hcol(r) for r in range(r0, r1, 8)])
    pre8 = pre8 + gb8 * y8
    wd_copy(n_wd - 1).wait()
    out8 = _tree_sum([wd_v[r:r + 8, :].astype(_F32) * hg_v[r - r_last:r - r_last + 8, :]
                      for r in range(r_last, _WD_SPLITS[-1], 8)] + [pre8])
    o_ref[...] = jnp.sum(out8, axis=0, keepdims=True).astype(o_ref.dtype)


@jax.jit
def pallas_adaLN_cond__compressed_kv_cla__glu_gated_geglu__decode_kernel(
    A_x: jax.Array,
    A_c_kv: jax.Array,
    A_w_q: jax.Array,
    A_w_uk: jax.Array,
    A_w_uv: jax.Array,
    A_w_o: jax.Array,
    B_x: jax.Array,
    B_w_gate: jax.Array,
    B_w_up: jax.Array,
    B_w_down: jax.Array,
    c: jax.Array,
    w_mod: jax.Array,
):
    del B_x
    B, SQ, M = A_x.shape
    SK, DC = A_c_kv.shape[1], A_c_kv.shape[2]
    H, D = A_w_q.shape[1], A_w_q.shape[2]
    assert B == 1 and SQ == 1 and c.shape[0] == 1
    assert B_w_down.shape[0] == _WD_SPLITS[-1]

    operands = (
        A_x.reshape(1, M),
        c,
        w_mod,
        A_w_q.reshape(M * H, D),
        A_w_uk.reshape(DC * H, D),
        A_c_kv.reshape(SK, DC),
        A_w_uv.reshape(DC * H, D),
        A_w_o.reshape(H * D, M),
        B_w_gate,
        B_w_up,
        B_w_down,
    )
    scratch = [pltpu.VMEM(a.shape, a.dtype) for a in operands] + [
        pltpu.VMEM((128, 128 * H), _BF16),
        pltpu.VMEM((H, DC), _BF16),
        pltpu.VMEM((H, DC), _F32),
        pltpu.VMEM((H, 128), _F32),
        pltpu.VMEM((H, 128), _F32),
        pltpu.VMEM((_WD_SPLITS[-1] - _VPU_ROW0, 128), _F32),
        pltpu.VMEM((_WD_SPLITS[-1] - _WD_SPLITS[-2], M), _F32),
    ]
    out = pl.pallas_call(
        functools.partial(_kernel, H=H, D=D, M=M, DC=DC, SK=SK),
        out_shape=jax.ShapeDtypeStruct((1, M), A_x.dtype),
        in_specs=[pl.BlockSpec(memory_space=pl.ANY)] * len(operands),
        out_specs=pl.BlockSpec(memory_space=pltpu.VMEM),
        scratch_shapes=scratch,
        compiler_params=pltpu.CompilerParams(vmem_limit_bytes=100 * 1024 * 1024),
    )(*operands)
    return out.reshape(B, SQ, M)
```

```python
import functools

import jax
import jax.numpy as jnp
from jax import lax
import jax.experimental.pallas as pl
import jax.experimental.pallas.tpu as pltpu

_NN = (((1,), (0,)), ((), ()))
_NT = (((1,), (1,)), ((), ()))
_F32 = jnp.float32
_BF16 = jnp.bfloat16

_KV_BLK = 64
_KV_RUN = 32
_TK = _KV_BLK * _KV_RUN
_STAGE_ROWS = 1008
_VPU_ROW0 = 1408

CFG = {'pieces': [('wo', 64), ('wo', 64), ('wo', 64), ('wo', 64), ('wo', 64), ('wo', 64), ('wo', 64),
            ('wo', 64), ('wo', 64), ('wo', 64), ('wo', 64), ('wo', 64), ('wo', 64), ('wo', 64),
            ('wo', 64), ('wo', 64), ('wo', 64), ('wo', 64), ('wo', 64), ('wo', 64), ('wo', 64),
            ('wo', 64), ('wo', 64), ('wd', 64), ('wd', 64), ('wd', 64), ('wd', 64)],
 'pat': (),
 'wd_splits': (1024, 1408, 1536, 1664, 1760, 1792),
 'wd_side_pos': 1,
 'script': {'start': '+kv0 h0 h1 h2 h3 +kv1 +wmod +x +c +kv2 +kv3 +wq +kv4 +kv5 +wuk +kv6 +kv7 '
                     '+kv8 +kv9 +kv10 +kv11 +kv12 +kv13 +kv14 +kv15 +wuv +wo',
            'mod': '!h3 s0 s1 s2 !wmod h4 h5 h6 h7',
            'q': '!h7 s3 s4 s5 s6 !wq h8 h9 h10 h11',
            'qa': '!h11 s7 s8 s9 s10 !wuk h12 h13 h14 h15 h16 h17 h18 h19 h20 h21 +wg +wu +wd0 '
                  '+wd1 +wd2 +wd3 +wd4 +wd5',
            'L0': 's11 h22 h23 h24 h25',
            'L4': 's12 h26',
            'L7': 's13',
            'L10': 's14',
            'L13': 's15',
            'L15': 's16 s17 s18 s19 s20 s21 s22 s23 s24',
            'uv': 's25 s26',
            'u': '!s23 !s24'}}


def _dot(a, b, dims=_NN):
    return lax.dot_general(a, b, dims, preferred_element_type=_F32)


def _layernorm(x, eps=1e-5):
    m = jnp.mean(x, axis=-1, keepdims=True)
    xc = x - m
    v = jnp.mean(xc * xc, axis=-1, keepdims=True)
    return xc / jnp.sqrt(v + eps)


def _tree_sum(parts):
    while len(parts) > 1:
        parts = [parts[i] + parts[i + 1] if i + 1 < len(parts) else parts[i]
                 for i in range(0, len(parts), 2)]
    return parts[0]


class _Copies:
    def __init__(self, sems):
        self.sems, self.defs, self.started, self.waited = sems, {}, set(), set()

    def define(self, name, pairs):
        self.defs[name] = (len(self.defs), pairs)

    def _descs(self, name):
        k, pairs = self.defs[name]
        return [pltpu.make_async_copy(s, d, self.sems.at[k]) for s, d in pairs]

    def start(self, name):
        assert name not in self.started, name
        self.started.add(name)
        for cp in self._descs(name):
            cp.start()

    def need(self, name):
        assert name in self.started, name
        if name not in self.waited:
            self.waited.add(name)
            for cp in self._descs(name):
                cp.wait()


def _n_sems(n_kv):
    return 9 + n_kv + len(CFG['wd_splits']) + 2 * len(CFG['pieces'])


def _kernel(*refs, n_kv, **dims):
    pl.run_scoped(lambda sems: _body(*refs, sems, n_kv=n_kv, **dims),
                  pltpu.SemaphoreType.DMA((_n_sems(n_kv),)))


def _body(x_hbm, c_hbm, wmod_hbm, wq_hbm, wuk_hbm, ckv_hbm, wuv_hbm, wo_hbm,
          wg_hbm, wu_hbm, wd_hbm,
          o_ref,
          x_v, c_v, wmod_v, wq_v, wuk_v, ckv_v, wuv_v, wo_v, wg_v, wu_v, wd_v,
          e_v, qa_v, acc_v, m_v, l_v, hcol_v, hg_v, stage_s, sems,
          *, H, D, M, DC, n_kv):
    G = 128 * H
    cps = _Copies(sems)
    script = CFG['script']
    pieces = CFG['pieces']

    hbm = dict(wo=wo_hbm, wd=wd_hbm)
    vm = dict(wo=wo_v, wd=wd_v)
    top = dict(wo=0, wd=0)
    span, pos = [], 0
    for k, (arr, rows) in enumerate(pieces):
        if pos + rows > _STAGE_ROWS:
            pos = 0
        r, s = pl.ds(top[arr], rows), pl.ds(pos, rows)
        cps.define('h%d' % k, [(hbm[arr].at[r], stage_s.at[s])])
        cps.define('s%d' % k, [(stage_s.at[s], vm[arr].at[r])])
        span.append((pos, pos + rows))
        top[arr] += rows
        pos += rows

    for name, src, dst in (('x', x_hbm, x_v), ('c', c_hbm, c_v), ('wg', wg_hbm, wg_v), ('wu', wu_hbm, wu_v)):
        cps.define(name, [(src, dst)])
    for name, src, dst in (('wmod', wmod_hbm, wmod_v), ('wq', wq_hbm, wq_v), ('wuk', wuk_hbm, wuk_v), ('wuv', wuv_hbm, wuv_v)):
        if name in CFG['pat']:
            cps.define(name, [(src.at[:, j], dst.at[:, j]) for j in range(src.shape[1])])
        else:
            cps.define(name, [(src, dst)])
    r = pl.ds(top['wo'], H * D - top['wo'])
    cps.define('wo', [(wo_hbm.at[r], wo_v.at[r])])
    for j in range(n_kv):
        cps.define('kv%d' % j, [(ckv_hbm.at[:, j], ckv_v.at[j])])
    wd_splits = (top['wd'],) + tuple(CFG['wd_splits'])
    n_wd = len(wd_splits) - 1
    for j in range(n_wd):
        r = pl.ds(wd_splits[j], wd_splits[j + 1] - wd_splits[j])
        cps.define('wd%d' % j, [(wd_hbm.at[r], wd_v.at[r])])

    def run(point):
        for op in script.get(point, '').split():
            if op[0] == '+':
                cps.start(op[1:])
            elif op[0] == '!':
                cps.need(op[1:])
            elif op[0] == 'h':
                k = int(op[1:])
                for e in range(k):
                    if span[e][0] < span[k][1] and span[k][0] < span[e][1]:
                        cps.need('s%d' % e)
                cps.start(op)
            elif op[0] == 's':
                cps.need('h' + op[1:])
                cps.start(op)

    run('start')

    CH = 1024
    for b in range(G // CH):
        row = lax.broadcasted_iota(jnp.int32, (128, CH), 0)
        col = lax.broadcasted_iota(jnp.int32, (128, CH), 1) + b * CH
        e_v[:, b * CH:(b + 1) * CH] = jnp.where(col // H == row, 1.0, 0.0).astype(_BF16)
    hsel = (lax.broadcasted_iota(jnp.int32, (H, CH), 1) % H
            == lax.broadcasted_iota(jnp.int32, (H, CH), 0))

    def wslab(w_ref, r0):
        blk, j0 = r0 // 2048, (r0 % 2048) // 128
        return w_ref[blk, j0:j0 + CH // 128].reshape(CH, D)

    def expand_contract(lhs, w_ref):
        out = jnp.zeros((H, D), _F32)
        for a in range(lhs.shape[1] // 128):
            la = lhs[:, a * 128:(a + 1) * 128]
            for b in range(G // CH):
                t = _dot(la, e_v[:, b * CH:(b + 1) * CH])
                t = jnp.where(hsel, t, 0.0).astype(_BF16)
                out = out + _dot(t, wslab(w_ref, a * G + b * CH))
        return out

    acc_v[...] = jnp.zeros_like(acc_v)
    m_v[...] = jnp.full_like(m_v, -jnp.inf)
    l_v[...] = jnp.zeros_like(l_v)

    run('mod')
    for n in ('wmod', 'x', 'c'):
        cps.need(n)
    c = c_v[...].astype(_F32)
    sc = (c * jax.nn.sigmoid(c)).astype(_BF16)
    mod = _dot(sc, wmod_v[...].reshape(M, 6 * M))
    sa, ca, ga, sb, cb, gb = [mod[:, i * M:(i + 1) * M] for i in range(6)]
    x = x_v[...].astype(_F32)
    h1 = (_layernorm(x) * (1.0 + ca) + sa).astype(_BF16)

    run('q')
    cps.need('wq')
    q = expand_contract(jnp.broadcast_to(h1, (H, M)), wq_v).astype(_BF16)

    run('qa')
    cps.need('wuk')
    scale = D ** (-0.5)
    for a in range(DC // 128):
        qa = jnp.zeros((H, 128), _F32)
        for b in range(G // CH):
            t = _dot(q, wslab(wuk_v, a * G + b * CH), _NT)
            t = jnp.where(hsel, t * scale, 0.0).astype(_BF16)
            qa = qa + _dot(t, e_v[:, b * CH:(b + 1) * CH], _NT)
        qa_v[:, a * 128:(a + 1) * 128] = qa.astype(_BF16)

    def attn_step(i, carry):
        for j in range(n_kv):
            if ('kv%d' % j) in cps.waited and not script.get('L%d' % j):
                continue

            @pl.when(i == j)
            def _(j=j):
                cps.need('kv%d' % j)
                run('L%d' % j)

        ck = ckv_v[i].reshape(_TK, DC)
        s = _dot(qa_v[...], ck, _NT)
        m_prev = m_v[...]
        m_new = jnp.maximum(m_prev, jnp.max(s, axis=1, keepdims=True))
        alpha = jnp.exp(m_prev - m_new)
        p = jnp.exp(s - m_new[:, 0:1])
        ps = p[:, 0:128]
        for j in range(1, _TK // 128):
            ps = ps + p[:, j * 128:(j + 1) * 128]
        l_v[...] = l_v[...] * alpha + ps
        m_v[...] = m_new
        acc_v[...] = acc_v[...] * alpha[:, 0:1] + _dot(p.astype(_BF16), ck)
        return carry

    lax.fori_loop(0, n_kv, attn_step, 0)

    l = jnp.sum(l_v[...], axis=1, keepdims=True)
    ctx_c = (acc_v[...] / l).astype(_BF16)

    run('uv')
    cps.need('wuv')
    run('uv2')
    ctx = expand_contract(ctx_c, wuv_v)

    rid = lax.broadcasted_iota(jnp.int32, (16, D), 0)
    blocks = []
    for h in range(H):
        g0 = (h // 16) * 16
        blocks.append(jnp.where(rid == h % 16, ctx[g0:g0 + 16, :], 0.0).astype(_BF16))
    ctx_bd = jnp.concatenate(blocks, axis=1)
    run('o')
    cps.need('wo')
    for k, (arr, _) in enumerate(pieces):
        if arr == 'wo':
            cps.need('s%d' % k)
    run('o2')
    attn = jnp.sum(_dot(ctx_bd, wo_v[...]), axis=0, keepdims=True)
    x1 = x + ga * attn

    h2 = (_layernorm(x1) * (1.0 + cb) + sb).astype(_BF16)
    run('g')
    cps.need('wg')
    g = jax.nn.gelu(_dot(h2, wg_v[...]), approximate=True)
    run('u')
    cps.need('wu')
    hh = (g * _dot(h2, wu_v[...])).astype(_BF16)

    DF = wd_splits[-1]
    for r in range(_VPU_ROW0, DF, 128):
        hcol_v[r - _VPU_ROW0:r - _VPU_ROW0 + 128, :] = jnp.transpose(
            jnp.broadcast_to(hh[:, r:r + 128].astype(_F32), (128, 128)))

    def hcol(r):
        hc = hcol_v[r - _VPU_ROW0:r - _VPU_ROW0 + 8, :]
        return jnp.concatenate([hc] * (M // 128), axis=1)

    gb8 = jnp.broadcast_to(gb, (8, M))
    r_last = wd_splits[-2]
    for r in range(r_last, DF, 8):
        hg_v[r - r_last:r - r_last + 8, :] = hcol(r) * gb8
    row0 = lax.broadcasted_iota(jnp.int32, (8, M), 0) == 0

    side128 = -(-top['wd'] // 128) * 128
    items = [(max(wd_splits[j], side128) if j == 0 else wd_splits[j], wd_splits[j + 1], ['wd%d' % j]) for j in range(n_wd - 1)]
    if side128:
        items.insert(CFG['wd_side_pos'], (0, side128, ['wd0'] + ['s%d' % k for k, (a, _) in enumerate(pieces) if a == 'wd']))
    y = None
    y8 = None
    for r0, r1, deps in items:
        for n in deps:
            cps.need(n)
        if r0 < _VPU_ROW0:
            t = _dot(hh[:, r0:r1], wd_v[r0:r1, :])
            y = t if y is None else t + y
        else:
            y8 = _tree_sum(([] if y8 is None else [y8]) + [
                wd_v[r:r + 8, :].astype(_F32) * hcol(r) for r in range(r0, r1, 8)])
    pre8 = jnp.where(row0, jnp.broadcast_to(x1 + gb * y, (8, M)), 0.0) + gb8 * y8
    cps.need('wd%d' % (n_wd - 1))
    out8 = _tree_sum([wd_v[r:r + 8, :].astype(_F32) * hg_v[r - r_last:r - r_last + 8, :]
                      for r in range(r_last, DF, 8)] + [pre8])
    o_ref[...] = jnp.sum(out8, axis=0, keepdims=True).astype(o_ref.dtype)
    assert cps.started == cps.waited == set(cps.defs), (set(cps.defs) - cps.started, cps.started - cps.waited)


@jax.jit
def pallas_adaLN_cond__compressed_kv_cla__glu_gated_geglu__decode_kernel(
    A_x, A_c_kv, A_w_q, A_w_uk, A_w_uv, A_w_o, B_x, B_w_gate, B_w_up, B_w_down, c, w_mod):
    del B_x
    B, SQ, M = A_x.shape
    SK, DC = A_c_kv.shape[1], A_c_kv.shape[2]
    H, D = A_w_q.shape[1], A_w_q.shape[2]
    n_kv = SK // _TK
    operands = (
        A_x.reshape(1, M),
        c,
        w_mod.reshape(2, 16, 16, 6 * M),
        A_w_q.reshape(8, 16, 128, D),
        A_w_uk.reshape(8, 16, 128, D),
        A_c_kv.reshape(_KV_BLK, n_kv, _KV_RUN, DC),
        A_w_uv.reshape(8, 16, 128, D),
        A_w_o.reshape(H * D, M),
        B_w_gate,
        B_w_up,
        B_w_down,
    )
    shapes = [a.shape for a in operands]
    shapes[5] = (n_kv, _KV_BLK, _KV_RUN, DC)
    DF = B_w_down.shape[0]
    scratch = [pltpu.VMEM(s, a.dtype) for s, a in zip(shapes, operands)] + [
        pltpu.VMEM((128, 128 * H), _BF16),
        pltpu.VMEM((H, DC), _BF16),
        pltpu.VMEM((H, DC), _F32),
        pltpu.VMEM((H, 128), _F32),
        pltpu.VMEM((H, 128), _F32),
        pltpu.VMEM((DF - _VPU_ROW0, 128), _F32),
        pltpu.VMEM((DF - CFG['wd_splits'][-2], M), _F32),
        pltpu.SMEM((_STAGE_ROWS, M), _BF16),
    ]
    out = pl.pallas_call(
        functools.partial(_kernel, H=H, D=D, M=M, DC=DC, n_kv=n_kv),
        out_shape=jax.ShapeDtypeStruct((1, M), A_x.dtype),
        in_specs=[pl.BlockSpec(memory_space=pl.ANY)] * len(operands),
        out_specs=pl.BlockSpec(memory_space=pltpu.VMEM),
        scratch_shapes=scratch,
        compiler_params=pltpu.CompilerParams(vmem_limit_bytes=100 * 1024 * 1024),
    )(*operands)
    return out.reshape(B, SQ, M)
```

```python
import functools

import jax
import jax.numpy as jnp
from jax import lax
import jax.experimental.pallas as pl
import jax.experimental.pallas.tpu as pltpu

_NN = (((1,), (0,)), ((), ()))
_NT = (((1,), (1,)), ((), ()))
_F32 = jnp.float32
_BF16 = jnp.bfloat16

_N_STRIDED = 16
_KV_RUN = 32
_W_RUN = 128

_PIECES = [('wo', 64)] * 11 + [('wo', 80)] + [('wo', 64)] * 11 + [('wd', 64)] * 4
_STAGE_ROWS = 784

_WD_ENDS = (1024, 1408, 1536, 1664, 1760, 1792)
_VPU_ROW0 = 1408
_WD_SIDE_POS = 1

_SCRIPT = {
    'start': '+kv0 h0 h1 h2 h3 +kv1 +wmod +x +c +wq',
    'mod': '!h3 s0 s1 s2 !wmod h4 h5 h6 h7 h8 h9 h10 h11 h12 h13 s3 +wuk',
    'q': '!wq s4 s5 h14 h15 ' + ' '.join('+kv%d' % j for j in range(2, _N_STRIDED)),
    'qa': '!wuk s6 s7 h16',
    'L2': 's8 h17 h18', 'L4': 's9 h19', 'L5': 's10 h20', 'L6': 's11 h21', 'L7': 's12 h22',
    'L8': 's13 h23', 'L9': 'h24 +wuv', 'L10': 's14 h25', 'L11': 's15', 'L12': 's16 h26',
    'L13': 's17 +wo +wg +wu', 'L14': 's18', 'L15': 's19',
    'uv': 's20 +wd0 +wd1 +wd2 +wd3 +wd4 +wd5 !wuv s21 s22 s23 s24 s25',
    'o': 's26',
    'u': '!s23 !s24',
}


def _plan():
    spans, tops, pos = [], dict(wo=0, wd=0), 0
    for arr, rows in _PIECES:
        if pos + rows > _STAGE_ROWS:
            pos = 0
        spans.append((pos, pos + rows))
        tops[arr] += rows
        pos += rows

    def side(a):
        return ['s%d' % k for k, (arr, _) in enumerate(_PIECES) if arr == a]

    tail = [['wd%d' % j] for j in range(len(_WD_ENDS))]
    tail.insert(_WD_SIDE_POS, side('wd'))
    points = ([('start', [], []), ('mod', [], ['wmod', 'x', 'c']), ('q', [], ['wq']),
               ('qa', [], ['wuk'])]
              + [('L%d' % j, ['kv%d' % j], []) for j in range(_N_STRIDED)]
              + [('uv', [], ['wuv']), ('o', [], ['wo'] + side('wo')), ('g', [], ['wg']),
                 ('u', [], ['wu'])]
              + [('T%d' % t, [], deps) for t, deps in enumerate(tail)])
    assert set(_SCRIPT) <= {p[0] for p in points}
    started, waited, ops = [], set(), {}
    for point, before, after in points:
        out = ops[point] = []

        def start(n):
            assert n not in started, n
            started.append(n)
            out.append(('start', n))

        def need(n):
            assert n in started, n
            if n not in waited:
                waited.add(n)
                out.append(('wait', n))

        for n in before:
            need(n)
        for op in _SCRIPT.get(point, '').split():
            if op[0] == '+':
                start(op[1:])
            elif op[0] == '!':
                need(op[1:])
            elif op[0] == 'h':
                k = int(op[1:])
                for e in range(k):
                    if spans[e][0] < spans[k][1] and spans[k][0] < spans[e][1]:
                        need('s%d' % e)
                start(op)
            else:
                assert op[0] == 's', op
                need('h' + op[1:])
                start(op)
        for n in after:
            need(n)
    assert set(started) == waited
    assert len(started) == 9 + _N_STRIDED + len(_WD_ENDS) + 2 * len(_PIECES)
    return started, spans, tops, ops


def _dot(a, b, dims=_NN):
    return lax.dot_general(a, b, dims, preferred_element_type=_F32)


def _layernorm(x, eps=1e-5):
    m = jnp.mean(x, axis=-1, keepdims=True)
    xc = x - m
    v = jnp.mean(xc * xc, axis=-1, keepdims=True)
    return xc / jnp.sqrt(v + eps)


def _tree_sum(parts):
    while len(parts) > 1:
        parts = [parts[i] + parts[i + 1] if i + 1 < len(parts) else parts[i]
                 for i in range(0, len(parts), 2)]
    return parts[0]


def _kernel(*refs, **dims):
    pl.run_scoped(lambda sems: _body(*refs, sems, **dims),
                  pltpu.SemaphoreType.DMA((len(_plan()[0]),)))


def _body(x_hbm, c_hbm, wmod_hbm, wq_hbm, wuk_hbm, ckv_hbm, wuv_hbm, wo_hbm,
          wg_hbm, wu_hbm, wd_hbm,
          o_ref,
          x_v, c_v, wmod_v, wq_v, wuk_v, ckv_v, wuv_v, wo_v, wg_v, wu_v, wd_v,
          e_v, qa_v, acc_v, m_v, l_v, hcol_v, hg_v, stage_s, sems,
          *, H, D, M, DC, TK):
    names, spans, tops, ops = _plan()

    pairs = {}
    for name, src, dst in (('x', x_hbm, x_v), ('c', c_hbm, c_v), ('wmod', wmod_hbm, wmod_v),
                           ('wg', wg_hbm, wg_v), ('wu', wu_hbm, wu_v)):
        pairs[name] = [(src, dst)]
    for name, src, dst in (('wq', wq_hbm, wq_v), ('wuk', wuk_hbm, wuk_v), ('wuv', wuv_hbm, wuv_v)):
        pairs[name] = [(src.at[:, j], dst.at[j]) for j in range(_N_STRIDED)]
    for j in range(_N_STRIDED):
        pairs['kv%d' % j] = [(ckv_hbm.at[:, j], ckv_v.at[j])]
    row = dict(wo=0, wd=0)
    for k, (arr, rows) in enumerate(_PIECES):
        src, dst = (wo_hbm, wo_v) if arr == 'wo' else (wd_hbm, wd_v)
        r, s = pl.ds(row[arr], rows), pl.ds(spans[k][0], rows)
        pairs['h%d' % k] = [(src.at[r], stage_s.at[s])]
        pairs['s%d' % k] = [(stage_s.at[s], dst.at[r])]
        row[arr] += rows
    r = pl.ds(tops['wo'], H * D - tops['wo'])
    pairs['wo'] = [(wo_hbm.at[r], wo_v.at[r])]
    wd_rows = list(zip((tops['wd'],) + _WD_ENDS[:-1], _WD_ENDS))
    for j, (r0, r1) in enumerate(wd_rows):
        pairs['wd%d' % j] = [(wd_hbm.at[pl.ds(r0, r1 - r0)], wd_v.at[pl.ds(r0, r1 - r0)])]

    def run(point):
        for what, name in ops[point]:
            for src, dst in pairs[name]:
                cp = pltpu.make_async_copy(src, dst, sems.at[names.index(name)])
                if what == 'start':
                    cp.start()
                else:
                    cp.wait()

    run('start')

    G = 128 * H
    CH = 1024
    for b in range(G // CH):
        rr = lax.broadcasted_iota(jnp.int32, (128, CH), 0)
        cc = lax.broadcasted_iota(jnp.int32, (128, CH), 1) + b * CH
        e_v[:, b * CH:(b + 1) * CH] = jnp.where(cc // H == rr, 1.0, 0.0).astype(_BF16)
    hsel = (lax.broadcasted_iota(jnp.int32, (H, CH), 1) % H
            == lax.broadcasted_iota(jnp.int32, (H, CH), 0))

    def wslab(w_ref, r0):
        blk, j0 = divmod(r0 // _W_RUN, _N_STRIDED)
        return w_ref[j0:j0 + CH // _W_RUN, blk].reshape(CH, D)

    def expand_contract(lhs, w_ref):
        out = jnp.zeros((H, D), _F32)
        for a in range(lhs.shape[1] // 128):
            la = lhs[:, a * 128:(a + 1) * 128]
            for b in range(G // CH):
                t = _dot(la, e_v[:, b * CH:(b + 1) * CH])
                t = jnp.where(hsel, t, 0.0).astype(_BF16)
                out = out + _dot(t, wslab(w_ref, a * G + b * CH))
        return out

    acc_v[...] = jnp.zeros_like(acc_v)
    m_v[...] = jnp.full_like(m_v, -jnp.inf)
    l_v[...] = jnp.zeros_like(l_v)

    run('mod')
    c = c_v[...].astype(_F32)
    sc = (c * jax.nn.sigmoid(c)).astype(_BF16)
    mod = _dot(sc, wmod_v[...])
    sa, ca, ga, sb, cb, gb = [mod[:, i * M:(i + 1) * M] for i in range(6)]
    x = x_v[...].astype(_F32)
    h1 = (_layernorm(x) * (1.0 + ca) + sa).astype(_BF16)

    run('q')
    q = expand_contract(jnp.broadcast_to(h1, (H, M)), wq_v).astype(_BF16)

    run('qa')
    scale = D ** (-0.5)
    for a in range(DC // 128):
        qa = jnp.zeros((H, 128), _F32)
        for b in range(G // CH):
            t = _dot(q, wslab(wuk_v, a * G + b * CH), _NT)
            t = jnp.where(hsel, t * scale, 0.0).astype(_BF16)
            qa = qa + _dot(t, e_v[:, b * CH:(b + 1) * CH], _NT)
        qa_v[:, a * 128:(a + 1) * 128] = qa.astype(_BF16)

    def attn_step(i, carry):
        for j in range(_N_STRIDED):
            pl.when(i == j)(functools.partial(run, 'L%d' % j))
        ck = ckv_v[i].reshape(TK, DC)
        s = _dot(qa_v[...], ck, _NT)
        m_prev = m_v[...]
        m_new = jnp.maximum(m_prev, jnp.max(s, axis=1, keepdims=True))
        alpha = jnp.exp(m_prev - m_new)
        p = jnp.exp(s - m_new[:, 0:1])
        ps = p[:, 0:128]
        for j in range(1, TK // 128):
            ps = ps + p[:, j * 128:(j + 1) * 128]
        l_v[...] = l_v[...] * alpha + ps
        m_v[...] = m_new
        acc_v[...] = acc_v[...] * alpha[:, 0:1] + _dot(p.astype(_BF16), ck)
        return carry

    lax.fori_loop(0, _N_STRIDED, attn_step, 0)

    l = jnp.sum(l_v[...], axis=1, keepdims=True)
    ctx_c = (acc_v[...] / l).astype(_BF16)

    run('uv')
    ctx = expand_contract(ctx_c, wuv_v)

    rid = lax.broadcasted_iota(jnp.int32, (16, D), 0)
    blocks = []
    for h in range(H):
        g0 = (h // 16) * 16
        blocks.append(jnp.where(rid == h % 16, ctx[g0:g0 + 16, :], 0.0).astype(_BF16))
    ctx_bd = jnp.concatenate(blocks, axis=1)
    run('o')
    attn = jnp.sum(_dot(ctx_bd, wo_v[...]), axis=0, keepdims=True)
    x1 = x + ga * attn

    h2 = (_layernorm(x1) * (1.0 + cb) + sb).astype(_BF16)
    run('g')
    g = jax.nn.gelu(_dot(h2, wg_v[...]), approximate=True)
    run('u')
    hh = (g * _dot(h2, wu_v[...])).astype(_BF16)

    DF = _WD_ENDS[-1]
    for r in range(_VPU_ROW0, DF, 128):
        hcol_v[r - _VPU_ROW0:r - _VPU_ROW0 + 128, :] = jnp.transpose(
            jnp.broadcast_to(hh[:, r:r + 128].astype(_F32), (128, 128)))

    def hcol(r):
        hc = hcol_v[r - _VPU_ROW0:r - _VPU_ROW0 + 8, :]
        return jnp.concatenate([hc] * (M // 128), axis=1)

    gb8 = jnp.broadcast_to(gb, (8, M))
    r_last = _WD_ENDS[-2]
    for r in range(r_last, DF, 8):
        hg_v[r - r_last:r - r_last + 8, :] = hcol(r) * gb8
    row0 = lax.broadcasted_iota(jnp.int32, (8, M), 0) == 0

    chunks = wd_rows[:-1]
    chunks.insert(_WD_SIDE_POS, (0, tops['wd']))
    y = None
    y8 = None
    for t_idx, (r0, r1) in enumerate(chunks):
        run('T%d' % t_idx)
        if r0 < _VPU_ROW0:
            t = _dot(hh[:, r0:r1], wd_v[r0:r1, :])
            y = t if y is None else t + y
        else:
            y8 = _tree_sum(([] if y8 is None else [y8]) + [
                wd_v[r:r + 8, :].astype(_F32) * hcol(r) for r in range(r0, r1, 8)])
    pre8 = jnp.where(row0, jnp.broadcast_to(x1 + gb * y, (8, M)), 0.0) + gb8 * y8
    run('T%d' % len(chunks))
    out8 = _tree_sum([wd_v[r:r + 8, :].astype(_F32) * hg_v[r - r_last:r - r_last + 8, :]
                      for r in range(r_last, DF, 8)] + [pre8])
    o_ref[...] = jnp.sum(out8, axis=0, keepdims=True).astype(o_ref.dtype)


@jax.jit
def pallas_adaLN_cond__compressed_kv_cla__glu_gated_geglu__decode_kernel(
    A_x: jax.Array,
    A_c_kv: jax.Array,
    A_w_q: jax.Array,
    A_w_uk: jax.Array,
    A_w_uv: jax.Array,
    A_w_o: jax.Array,
    B_x: jax.Array,
    B_w_gate: jax.Array,
    B_w_up: jax.Array,
    B_w_down: jax.Array,
    c: jax.Array,
    w_mod: jax.Array,
):
    del B_x
    B, SQ, M = A_x.shape
    SK, DC = A_c_kv.shape[1], A_c_kv.shape[2]
    H, D = A_w_q.shape[1], A_w_q.shape[2]
    DF = B_w_down.shape[0]
    assert B == 1 and SQ == 1 and c.shape[0] == 1 and DF == _WD_ENDS[-1]

    operands = (
        A_x.reshape(1, M),
        c,
        w_mod,
        A_w_q.reshape(-1, _N_STRIDED, _W_RUN, D),
        A_w_uk.reshape(-1, _N_STRIDED, _W_RUN, D),
        A_c_kv.reshape(-1, _N_STRIDED, _KV_RUN, DC),
        A_w_uv.reshape(-1, _N_STRIDED, _W_RUN, D),
        A_w_o.reshape(H * D, M),
        B_w_gate,
        B_w_up,
        B_w_down,
    )

    def vmem_like(a):
        shape = a.shape if a.ndim == 2 else (a.shape[1], a.shape[0]) + a.shape[2:]
        return pltpu.VMEM(shape, a.dtype)

    scratch = [vmem_like(a) for a in operands] + [
        pltpu.VMEM((128, 128 * H), _BF16),
        pltpu.VMEM((H, DC), _BF16),
        pltpu.VMEM((H, DC), _F32),
        pltpu.VMEM((H, 128), _F32),
        pltpu.VMEM((H, 128), _F32),
        pltpu.VMEM((DF - _VPU_ROW0, 128), _F32),
        pltpu.VMEM((DF - _WD_ENDS[-2], M), _F32),
        pltpu.SMEM((_STAGE_ROWS, M), _BF16),
    ]
    out = pl.pallas_call(
        functools.partial(_kernel, H=H, D=D, M=M, DC=DC, TK=SK // _N_STRIDED),
        out_shape=jax.ShapeDtypeStruct((1, M), A_x.dtype),
        in_specs=[pl.BlockSpec(memory_space=pl.ANY)] * len(operands),
        out_specs=pl.BlockSpec(memory_space=pltpu.VMEM),
        scratch_shapes=scratch,
        compiler_params=pltpu.CompilerParams(vmem_limit_bytes=100 * 1024 * 1024),
    )(*operands)
    return out.reshape(B, SQ, M)
```
